```python
import jax
import jax.numpy as jnp

def _softmax(x, axis=-1):
    return jax.nn.softmax(x, axis=axis)
def _gelu(x):
    return jax.nn.gelu(x, approximate=True)
def _silu(x):
    return jax.nn.silu(x)
def _sigmoid(x):
    return jax.nn.sigmoid(x)
def _layernorm(x, axis=-1, eps=1e-5):
    m = jnp.mean(x, axis=axis, keepdims=True)
    v = jnp.var(x, axis=axis, keepdims=True)
    return (x - m) / jnp.sqrt(v + eps)
def _scatter_add(tgt, idx, src, axis=0):
    return tgt.at[idx].add(src)
def _segment_sum(src, seg, n):
    return jax.ops.segment_sum(src, seg, n)
class _Rng:
    def __init__(self, key):
        self._k = key
    def _next(self):
        self._k, sub = jax.random.split(self._k)
        return sub
    def normal(self, shape):
        return jax.random.normal(self._next(), shape, dtype=jnp.bfloat16)
    def randint(self, lo, hi, shape):
        return jax.random.randint(self._next(), shape, lo, hi, dtype=jnp.int32)
    def uniform(self, shape, lo=0.0, hi=1.0):
        return jax.random.uniform(self._next(), shape, jnp.bfloat16, lo, hi)
    def permutation(self, n):
        return jax.random.permutation(self._next(), n)


kernel_name = 'sequential_preLN__sliding_local_dilated__moe_arch_mod__prompt'

def setup_inputs():
    _rng = _Rng(jax.random.key(int.from_bytes(__import__("os").urandom(4), "little")))
    _w = (lambda a: (lambda t: t.astype(jnp.bfloat16) if jnp.issubdtype(t.dtype, jnp.floating) else t)(jnp.asarray(a)))
    def _A_setup():
        B, S, D = 1, 2048, 640
        return {
            "x": _w((lambda *s: _rng.normal(s) * 0.05)(B, S, D)),
            "wqkv": _w((lambda *s: _rng.normal(s) * 0.05)(D, 3 * D)),
            "wo": _w((lambda *s: _rng.normal(s) * 0.05)(D, D)),
        }
    _A_in = _A_setup()

    def _B_setup():
        B, S, D, F, C = 1, 2048, 640, 1536, 1
        return {
            "x": _w((lambda *s: _rng.normal(s) * 0.05)(B, S, D)),
            "w_r": _w((lambda *s: _rng.normal(s) * 0.05)(D)),
            "w_gate": _w((lambda *s: _rng.normal(s) * 0.05)(D, F)),
            "w_up": _w((lambda *s: _rng.normal(s) * 0.05)(D, F)),
            "w_down": _w((lambda *s: _rng.normal(s) * 0.05)(F, D)),
        }
    _B_in = _B_setup()

    return {
        "A_x": _A_in["x"],
        "A_wqkv": _A_in["wqkv"],
        "A_wo": _A_in["wo"],
        "B_x": _B_in["x"],
        "B_w_r": _B_in["w_r"],
        "B_w_gate": _B_in["w_gate"],
        "B_w_up": _B_in["w_up"],
        "B_w_down": _B_in["w_down"],
    }

def reference(A_x, A_wqkv, A_wo, B_x, B_w_r, B_w_gate, B_w_up, B_w_down):
    def _A_ref(x, wqkv, wo):
        B, S, D = x.shape
        H = 32; Dh = D // H
        W, dil = 8, 2
        qkv = (lambda x, *d: x.transpose(*d))((x @ wqkv).reshape(B, S, 3, H, Dh), 2, 0, 3, 1, 4)
        q, k, v = qkv[0], qkv[1], qkv[2]
        scale = Dh ** -0.5
        pos = jnp.arange(S)
        off = jnp.arange(W) * dil
        idx = pos[:, None] - off[None, :]
        mask = idx >= 0
        idx_c = jnp.where(mask, idx, 0).reshape(-1)
        kg = k[:, :, idx_c, :].reshape(B, H, S, W, Dh)
        vg = v[:, :, idx_c, :].reshape(B, H, S, W, Dh)
        logits = jnp.einsum("bhsd,bhswd->bhsw", q, kg) * scale
        logits = jnp.where(mask[None, None, :, :], logits, -1e9)
        attn = _softmax(logits, axis=-1)
        o = jnp.einsum("bhsw,bhswd->bhsd", attn, vg)
        return (lambda x, *d: x.transpose(*d))(o, 0, 2, 1, 3).reshape(B, S, D) @ wo

    def _B_ref(x, w_r, w_gate, w_up, w_down):
        B, S, D = x.shape
        C = 1
        r = x @ w_r
        idx = jnp.argsort(-r, axis=-1)[:, :C]
        idx_e = jnp.repeat(idx.reshape(B, C, 1), D, axis=2)
        x_sel = jnp.take_along_axis(x, idx_e, axis=1)
        g = _silu(x_sel @ w_gate)
        u = x_sel @ w_up
        y = (g * u) @ w_down
        r_sel = _sigmoid(jnp.take_along_axis(r, idx, axis=1))
        y = y * r_sel.reshape(B, C, 1)
        b_off = (jnp.arange(B) * S).reshape(B, 1)
        flat_idx = (idx + b_off).reshape(B * C)
        zero = (x * 0.0).reshape(B * S, D)
        upd = _scatter_add(zero, flat_idx, y.reshape(B * C, D), axis=0)
        return x + upd.reshape(B, S, D)

    x = A_x
    h = x + _A_ref(_layernorm(x, axis=-1), A_wqkv, A_wo)
    h2 = h + _B_ref(_layernorm(h, axis=-1), B_w_r, B_w_gate, B_w_up, B_w_down)
    return h2
```

```python
import functools
import jax
import jax.numpy as jnp
import numpy as np
from jax.experimental import pallas as pl
from jax.experimental.pallas import tpu as pltpu

S, D, H, DH, F = 2048, 640, 32, 20, 1536
WIN, DIL = 8, 2
NT = D // 128
HALO = 16
EPS = 1e-5
LOG2E = 1.4426950408889634
QSCALE = float(DH ** -0.5) * LOG2E
NEG = -1e9 * LOG2E
bf16 = jnp.bfloat16
f32 = jnp.float32
u32 = jnp.uint32


def _ln(x):
    m = jnp.sum(x, axis=1, keepdims=True) * (1.0 / D)
    c = x - m
    v = jnp.sum(c * c, axis=1, keepdims=True) * (1.0 / D)
    return c * jax.lax.rsqrt(v + EPS)


def _permute_rows(tmp, store):
    for kt in range(NT):
        for dd in range(DH // 2):
            for g in range(2):
                a = tmp[kt, pl.ds(g * 160 + dd, 8, stride=20), :]
                b = tmp[kt, pl.ds(g * 160 + dd + 10, 8, stride=20), :]
                lo = (a & jnp.uint32(0xFFFF)) | (b << 16)
                hi = (a >> 16) | (b & jnp.uint32(0xFFFF0000))
                store(kt, (2 * dd) * 32 + g * 16, pltpu.bitcast(lo, bf16))
                store(kt, (2 * dd + 1) * 32 + g * 16, pltpu.bitcast(hi, bf16))


def make(BM=256, RC=16, lagC=1, lagD=1):
    NB = S // BM

    def kernel(x_hbm, wqkv_hbm, wo_hbm, wr_ref, wg_hbm, wu_hbm, wd_hbm, out_hbm,
               x_v, wqkv_v, wo_v, wg_v, wu_v, wd_v, out_v, patch_v,
               tmp, wp, wop, xn_s, q_s, k_s, v_s, o_s, h_s,
               sem_x, sem_w, sem_o, sem_p):
        def cp_x(i):
            return pltpu.make_async_copy(x_hbm.at[pl.ds(i * BM, BM)], x_v.at[pl.ds(i * BM, BM)], sem_x.at[i])

        def cp_w(t):
            return pltpu.make_async_copy(wqkv_hbm.at[:, pl.ds(t * D, D)], wqkv_v.at[:, pl.ds(t * D, D)], sem_w.at[t])

        cp_wo = pltpu.make_async_copy(wo_hbm, wo_v, sem_w.at[3])
        cp_wg = pltpu.make_async_copy(wg_hbm, wg_v, sem_w.at[4])
        cp_wu = pltpu.make_async_copy(wu_hbm, wu_v, sem_w.at[5])
        cp_wd = pltpu.make_async_copy(wd_hbm, wd_v, sem_w.at[6])

        def cp_o(i):
            return pltpu.make_async_copy(out_v.at[pl.ds(i * BM, BM)], out_hbm.at[pl.ds(i * BM, BM)], sem_o.at[i])

        cp_w(0).start()
        cp_x(0).start()
        cp_w(1).start()
        cp_w(2).start()
        for i in range(1, NB):
            cp_x(i).start()
        cp_wo.start()
        cp_wg.start()
        cp_wu.start()
        cp_wd.start()

        for t in range(NT):
            k_s[t, pl.ds(0, HALO), :] = jnp.zeros((HALO, 128), f32)
            v_s[t, pl.ds(0, HALO), :] = jnp.zeros((HALO, 128), f32)

        wr = wr_ref[...].astype(f32).reshape(1, D)

        def prep_w(t):
            cp_w(t).wait()
            for kt in range(NT):
                blk = wqkv_v[pl.ds(kt * 128, 128), pl.ds(t * D, D)]
                tmp[t, kt] = pltpu.bitcast(blk.T, u32)

            def store(kt, r, val):
                wp[pl.ds(t * D + r, 16), pl.ds(kt * 128, 128)] = val
            _permute_rows(tmp.at[t], store)

        def prep_wo():
            cp_wo.wait()
            for kt in range(NT):
                tmp[3, kt] = pltpu.bitcast(wo_v[:, pl.ds(kt * 128, 128)], u32)

            def store(kt, r, val):
                wop[pl.ds(r, 16), pl.ds(kt * 128, 128)] = val
            _permute_rows(tmp.at[3], store)

        def stage_ln(i):
            cp_x(i).wait()
            for c in range(BM // RC):
                r0 = i * BM + c * RC
                xx = x_v[pl.ds(r0, RC), :].astype(f32)
                xn_s[pl.ds(r0, RC), :] = _ln(xx).astype(bf16)

        def stage_a(i):
            xn = xn_s[pl.ds(i * BM, BM), :]
            for t3, dst in enumerate((q_s, k_s, v_s)):
                res = jax.lax.dot_general(xn, wp[pl.ds(t3 * D, D), :], (((1,), (1,)), ((), ())),
                                          preferred_element_type=f32)
                if t3 == 0:
                    res = res * QSCALE
                off = 0 if t3 == 0 else HALO
                for t in range(NT):
                    dst[t, pl.ds(off + i * BM, BM), :] = res[:, t * 128:(t + 1) * 128]

        def stage_b(i):
            for c in range(BM // RC):
                r0 = i * BM + c * RC
                q = [q_s[t, pl.ds(r0, RC), :] for t in range(NT)]
                L = []
                for j in range(WIN):
                    acc = None
                    for t in range(NT):
                        p = q[t] * k_s[t, pl.ds(HALO + r0 - DIL * j, RC), :]
                        acc = p if acc is None else acc + p
                    acc = acc + pltpu.roll(acc, 64, 1)
                    acc = acc + pltpu.roll(acc, 32, 1)
                    if r0 < DIL * j:
                        row = jax.lax.broadcasted_iota(jnp.int32, (RC, 128), 0) + r0
                        acc = jnp.where(row >= DIL * j, acc, NEG)
                    L.append(acc)
                m = L[0]
                for j in range(1, WIN):
                    m = jnp.maximum(m, L[j])
                e = [jnp.exp2(l - m) for l in L]
                ssum = e[0]
                for j in range(1, WIN):
                    ssum = ssum + e[j]
                inv = 1.0 / ssum
                for t in range(NT):
                    acc = None
                    for j in range(WIN):
                        p = e[j] * v_s[t, pl.ds(HALO + r0 - DIL * j, RC), :]
                        acc = p if acc is None else acc + p
                    o_s[pl.ds(r0, RC), pl.ds(t * 128, 128)] = (acc * inv).astype(bf16)

        def stage_c(i):
            o = o_s[pl.ds(i * BM, BM), :]
            res = jnp.dot(o, wop[...], preferred_element_type=f32)
            h_s[pl.ds(i * BM, BM), :] = res + x_v[pl.ds(i * BM, BM), :].astype(f32)

        best = [None, None]

        def stage_d(i):
            for c in range(BM // RC):
                r0 = i * BM + c * RC
                hh = h_s[pl.ds(r0, RC), :]
                xn2 = _ln(hh)
                out_v[pl.ds(r0, RC), :] = (hh + xn2).astype(bf16)
                r = jnp.sum(xn2 * wr, axis=1, keepdims=True)
                if best[0] is None:
                    best[0] = r
                    best[1] = jnp.full((RC, 1), float(r0), f32)
                else:
                    upd = r > best[0]
                    best[0] = jnp.where(upd, r, best[0])
                    best[1] = jnp.where(upd, float(r0), best[1])
            cp_o(i).start()

        stage_ln(0)
        prep_w(0); prep_w(1); prep_w(2)
        stage_a(0)
        stage_ln(1)
        prep_wo()
        nit = NB + lagC + lagD
        for it in range(nit):
            if it + 1 < NB:
                stage_a(it + 1)
            if it + 2 < NB:
                stage_ln(it + 2)
            if it < NB:
                stage_b(it)
            if 0 <= it - lagC < NB:
                stage_c(it - lagC)
            if 0 <= it - lagC - lagD < NB:
                stage_d(it - lagC - lagD)

        m = jnp.max(best[0], axis=0, keepdims=True)
        rowi = jax.lax.broadcasted_iota(jnp.int32, (RC, 1), 0).astype(f32)
        cand = jnp.where(best[0] == m, best[1] + rowi, float(S))
        idx = jnp.min(cand).astype(jnp.int32)
        idx = jnp.clip(idx, 0, S - 1)
        base = pl.multiple_of((idx // 16) * 16, 16)
        hh = h_s[pl.ds(base, 16), :]
        xn2 = _ln(hh)
        r = jnp.sum(xn2 * wr, axis=1, keepdims=True)
        xb = xn2.astype(bf16)
        cp_wg.wait(); cp_wu.wait(); cp_wd.wait()
        g = jnp.dot(xb, wg_v[...], preferred_element_type=f32)
        u = jnp.dot(xb, wu_v[...], preferred_element_type=f32)
        a = (g * jax.nn.sigmoid(g) * u).astype(bf16)
        y = jnp.dot(a, wd_v[...], preferred_element_type=f32)
        y = y * jax.nn.sigmoid(r)
        rowsel = jax.lax.broadcasted_iota(jnp.int32, (16, D), 0) == (idx - base)
        patch_v[...] = (hh + xn2 + jnp.where(rowsel, y, 0.0)).astype(bf16)
        for i in range(NB):
            cp_o(i).wait()
        cp = pltpu.make_async_copy(patch_v, out_hbm.at[pl.ds(base, 16)], sem_p)
        cp.start()
        cp.wait()

    scratch = [
        pltpu.VMEM((S, D), bf16), pltpu.VMEM((D, 3 * D), bf16), pltpu.VMEM((D, D), bf16),
        pltpu.VMEM((D, F), bf16), pltpu.VMEM((D, F), bf16), pltpu.VMEM((F, D), bf16),
        pltpu.VMEM((S, D), bf16), pltpu.VMEM((16, D), bf16),
        pltpu.VMEM((4, NT, 320, 128), u32), pltpu.VMEM((3 * D, D), bf16), pltpu.VMEM((D, D), bf16),
        pltpu.VMEM((S, D), bf16), pltpu.VMEM((NT, S, 128), f32),
        pltpu.VMEM((NT, HALO + S, 128), f32), pltpu.VMEM((NT, HALO + S, 128), f32),
        pltpu.VMEM((S, D), bf16), pltpu.VMEM((S, D), f32),
        pltpu.SemaphoreType.DMA((NB,)), pltpu.SemaphoreType.DMA((7,)), pltpu.SemaphoreType.DMA((NB,)),
        pltpu.SemaphoreType.DMA(()),
    ]
    any_spec = pl.BlockSpec(memory_space=pl.ANY)

    def fn(A_x, A_wqkv, A_wo, B_x, B_w_r, B_w_gate, B_w_up, B_w_down):
        out = pl.pallas_call(
            kernel,
            out_shape=jax.ShapeDtypeStruct((S, D), bf16),
            in_specs=[any_spec, any_spec, any_spec, pl.BlockSpec(memory_space=pltpu.VMEM), any_spec, any_spec, any_spec],
            out_specs=any_spec,
            scratch_shapes=scratch,
            compiler_params=pltpu.CompilerParams(vmem_limit_bytes=100 * 2 ** 20),
        )(A_x.reshape(S, D), A_wqkv, A_wo, B_w_r, B_w_gate, B_w_up, B_w_down)
        return out.reshape(1, S, D)
    return fn


_fn = make()


@jax.jit
def pallas_sequential_preLN__sliding_local_dilated__moe_arch_mod__prompt_kernel(
    A_x, A_wqkv, A_wo, B_x, B_w_r, B_w_gate, B_w_up, B_w_down,
):
    return _fn(A_x, A_wqkv, A_wo, B_x, B_w_r, B_w_gate, B_w_up, B_w_down)
```

```python
import functools
import jax
import jax.numpy as jnp
import numpy as np
from jax.experimental import pallas as pl
from jax.experimental.pallas import tpu as pltpu

S, D, H, DH, F = 2048, 640, 32, 20, 1536
WIN, DIL = 8, 2
NT = D // 128
HALO = 16
EPS = 1e-5
LOG2E = 1.4426950408889634
QSCALE = float(DH ** -0.5) * LOG2E
NEG = -1e9 * LOG2E
bf16 = jnp.bfloat16
f32 = jnp.float32
u32 = jnp.uint32


def _ln(x):
    m = jnp.sum(x, axis=1, keepdims=True) * (1.0 / D)
    c = x - m
    v = jnp.sum(c * c, axis=1, keepdims=True) * (1.0 / D)
    return c * jax.lax.rsqrt(v + EPS)


def _permute_rows(tmp, store):
    for kt in range(NT):
        for dd in range(DH // 2):
            for g in range(2):
                a = tmp[kt, pl.ds(g * 160 + dd, 8, stride=20), :]
                b = tmp[kt, pl.ds(g * 160 + dd + 10, 8, stride=20), :]
                lo = (a & jnp.uint32(0xFFFF)) | (b << 16)
                hi = (a >> 16) | (b & jnp.uint32(0xFFFF0000))
                store(kt, (2 * dd) * 16 + g * 8, lo)
                store(kt, (2 * dd + 1) * 16 + g * 8, hi)


def make(BM=256, RC=16, RCL=16, RCD=16, order=None, lagC=1, lagD=1):
    NB = S // BM

    def kernel(x_hbm, wqkv_hbm, wo_hbm, wr_ref, wg_hbm, wu_hbm, wd_hbm, out_hbm, *scr):
        scr = list(scr)
        def take(n):
            r = scr[:n]; del scr[:n]; return r
        wqkv_v, wo_v, wg_v, wu_v, wd_v, patch_v, tile_v, tmp, wp, wop = take(10)
        x_v = take(NB); out_v = take(NB); xn_s = take(NB); q_s = take(NB); k_s = take(NB); v_s = take(NB)
        o_s = take(NB); h_s = take(NB)
        sem_x, sem_w, sem_o, sem_p = take(4)

        def cp_x(i):
            return pltpu.make_async_copy(x_hbm.at[pl.ds(i * BM, BM)], x_v[i], sem_x.at[i])

        def cp_w(t):
            return pltpu.make_async_copy(wqkv_hbm.at[:, pl.ds(t * D, D)], wqkv_v.at[:, pl.ds(t * D, D)], sem_w.at[t])

        cp_wo = pltpu.make_async_copy(wo_hbm, wo_v, sem_w.at[3])
        cp_wg = pltpu.make_async_copy(wg_hbm, wg_v, sem_w.at[4])
        cp_wu = pltpu.make_async_copy(wu_hbm, wu_v, sem_w.at[5])
        cp_wd = pltpu.make_async_copy(wd_hbm, wd_v, sem_w.at[6])

        def cp_o(i):
            return pltpu.make_async_copy(out_v[i], out_hbm.at[pl.ds(i * BM, BM)], sem_o.at[i])

        cp_w(0).start()
        cp_x(0).start()
        cp_w(1).start()
        cp_w(2).start()
        for i in range(1, NB):
            cp_x(i).start()
        cp_wo.start()
        cp_wg.start()
        cp_wu.start()
        cp_wd.start()

        for t in range(NT):
            k_s[0][t, pl.ds(0, HALO), :] = jnp.zeros((HALO, 128), f32)
            v_s[0][t, pl.ds(0, HALO), :] = jnp.zeros((HALO, 128), f32)

        wr = wr_ref[...].astype(f32).reshape(1, D)

        def prep_w(t):
            cp_w(t).wait()
            for kt in range(NT):
                blk = wqkv_v[pl.ds(kt * 128, 128), pl.ds(t * D, D)]
                tmp[t, kt] = pltpu.bitcast(blk.T, u32)

            def store(kt, r, val):
                wp[t, kt, pl.ds(r, 8), :] = val
            _permute_rows(tmp.at[t], store)

        def prep_wo():
            cp_wo.wait()
            for kt in range(NT):
                tmp[3, kt] = pltpu.bitcast(wo_v[:, pl.ds(kt * 128, 128)], u32)

            def store(kt, r, val):
                wop[kt, pl.ds(r, 8), :] = val
            _permute_rows(tmp.at[3], store)

        def stage_ln(i):
            cp_x(i).wait()
            stage_ln_chunks(i, range(BM // RCL))

        def stage_ln_chunks(i, cs):
            for c in cs:
                r0 = c * RCL
                xx = x_v[i][pl.ds(r0, RCL), :].astype(f32)
                xn = _ln(xx).astype(bf16)
                for t in range(NT):
                    xn_s[i][t, pl.ds(r0 // 2, RCL // 2), :] = pltpu.bitcast(xn[:, t * 128:(t + 1) * 128], u32)

        def cat(ref, *idx):
            ps = [ref[(*idx, t)] for t in range(NT)]
            ps = [pltpu.bitcast(p, bf16) if p.dtype == u32 else p.astype(bf16) for p in ps]
            return jnp.concatenate(ps, axis=1)

        def stage_a(i, t3):
            xn = cat(xn_s[i])
            dst = (q_s, k_s, v_s)[t3]
            res = jax.lax.dot_general(xn, cat(wp, t3), (((1,), (1,)), ((), ())), preferred_element_type=f32)
            for t in range(NT):
                if t3 == 0:
                    dst[i][t] = res[:, t * 128:(t + 1) * 128]
                else:
                    dst[i][t, pl.ds(HALO, BM), :] = res[:, t * 128:(t + 1) * 128]
                    if i + 1 < NB:
                        dst[i + 1][t, pl.ds(0, HALO), :] = res[BM - HALO:, t * 128:(t + 1) * 128]

        def b1(i, r0):
            q = [q_s[i][t, pl.ds(r0, RC), :] for t in range(NT)]
            accs = []
            for j in range(WIN):
                acc = None
                for t in range(NT):
                    p = q[t] * k_s[i][t, pl.ds(HALO + r0 - DIL * j, RC), :]
                    acc = p if acc is None else acc + p
                accs.append(acc)
            return [(a, pltpu.roll(a, 64, 1)) for a in accs]

        def b2(st):
            out = []
            for (a, r) in st:
                s = a + r
                out.append((s, pltpu.roll(s, 32, 1)))
            return out

        def b3(i, r0, st):
            L = []
            for j in range(WIN):
                acc = (st[j][0] + st[j][1]) * QSCALE
                if i * BM + r0 < DIL * j:
                    row = jax.lax.broadcasted_iota(jnp.int32, (RC, 128), 0) + (i * BM + r0)
                    acc = jnp.where(row >= DIL * j, acc, NEG)
                L.append(acc)
            m = L[0]
            for j in range(1, WIN):
                m = jnp.maximum(m, L[j])
            e = [jnp.exp2(l - m) for l in L]
            ssum = e[0]
            for j in range(1, WIN):
                ssum = ssum + e[j]
            inv = 1.0 / ssum
            for t in range(NT):
                acc = None
                for j in range(WIN):
                    p = e[j] * v_s[i][t, pl.ds(HALO + r0 - DIL * j, RC), :]
                    acc = p if acc is None else acc + p
                if RC == 8:
                    o_s[i][t, pl.ds(r0, RC), :] = acc * inv
                else:
                    o_s[i][t, pl.ds(r0 // 2, RC // 2), :] = pltpu.bitcast((acc * inv).astype(bf16), u32)

        s1 = {}; s2 = {}
        ncb = BM // RC
        def b_step(g):
            n = NB * ncb
            if 0 <= g < n:
                s1[g] = b1(g // ncb, (g % ncb) * RC)
            if 0 <= g - 1 < n:
                s2[g - 1] = b2(s1.pop(g - 1))
            if 0 <= g - 2 < n:
                b3((g - 2) // ncb, ((g - 2) % ncb) * RC, s2.pop(g - 2))

        def stage_c(i):
            res = jnp.dot(cat(o_s[i]), cat(wop), preferred_element_type=f32)
            h_s[i][...] = res + x_v[i][...].astype(f32)

        best = [None, None]

        def stage_d(i, cs):
            for c in cs:
                r0 = c * RCD
                hh = h_s[i][pl.ds(r0, RCD), :]
                xn2 = _ln(hh)
                out_v[i][pl.ds(r0, RCD), :] = (hh + xn2).astype(bf16)
                r = jnp.sum(xn2 * wr, axis=1, keepdims=True)
                g0 = float(i * BM + r0)
                if best[0] is None:
                    best[0] = r
                    best[1] = jnp.full((RCD, 1), g0, f32)
                else:
                    upd = r > best[0]
                    best[0] = jnp.where(upd, r, best[0])
                    best[1] = jnp.where(upd, g0, best[1])

        stage_ln(0)
        prep_w(0); stage_a(0, 0)
        prep_w(1); stage_a(0, 1)
        prep_w(2); stage_a(0, 2)
        stage_ln(1)
        prep_wo()
        nit = NB + lagC + lagD
        nl = BM // RCL; nd = BM // RCD
        gb = 0
        for it in range(nit):
            for sl in range(4):
                mm = (lambda: stage_a(it + 1, sl)) if sl < 3 else (lambda: stage_c(it - lagC))
                do_mm = (it + 1 < NB) if sl < 3 else (0 <= it - lagC < NB)
                def vpu():
                    nonlocal gb
                    tgt = min((it * 4 + sl + 1) * (ncb // 4), NB * ncb + 2)
                    if it == NB - 1 and sl == 3:
                        tgt = NB * ncb + 2
                    while gb < tgt:
                        b_step(gb); gb += 1
                    if it + 2 < NB:
                        if sl == 0:
                            cp_x(it + 2).wait()
                        stage_ln_chunks(it + 2, range(sl * nl // 4, (sl + 1) * nl // 4))
                    j = it - lagC - lagD
                    if 0 <= j < NB:
                        stage_d(j, range(sl * nd // 4, (sl + 1) * nd // 4))
                        if sl == 3:
                            cp_o(j).start()
                if order == 'mm_first':
                    if do_mm: mm()
                    vpu()
                else:
                    vpu()
                    if do_mm: mm()

        m = jnp.max(best[0], axis=0, keepdims=True)
        rowi = jax.lax.broadcasted_iota(jnp.int32, (RCD, 1), 0).astype(f32)
        cand = jnp.where(best[0] == m, best[1] + rowi, float(S))
        idx = jnp.min(cand).astype(jnp.int32)
        idx = jnp.clip(idx, 0, S - 1)
        base = pl.multiple_of((idx // 16) * 16, 16)
        blk = idx // BM
        lbase = pl.multiple_of(base - blk * BM, 16)
        for b in range(NB):
            @pl.when(blk == b)
            def _():
                tile_v[...] = h_s[b][pl.ds(lbase, 16), :]
        hh = tile_v[...]
        xn2 = _ln(hh)
        r = jnp.sum(xn2 * wr, axis=1, keepdims=True)
        xb = xn2.astype(bf16)
        cp_wg.wait(); cp_wu.wait(); cp_wd.wait()
        g = jnp.dot(xb, wg_v[...], preferred_element_type=f32)
        u = jnp.dot(xb, wu_v[...], preferred_element_type=f32)
        a = (g * jax.nn.sigmoid(g) * u).astype(bf16)
        y = jnp.dot(a, wd_v[...], preferred_element_type=f32)
        y = y * jax.nn.sigmoid(r)
        rowsel = jax.lax.broadcasted_iota(jnp.int32, (16, D), 0) == (idx - base)
        patch_v[...] = (hh + xn2 + jnp.where(rowsel, y, 0.0)).astype(bf16)
        for i in range(NB):
            cp_o(i).wait()
        cp = pltpu.make_async_copy(patch_v, out_hbm.at[pl.ds(base, 16)], sem_p)
        cp.start()
        cp.wait()

    V = pltpu.VMEM
    scratch = [
        V((D, 3 * D), bf16), V((D, D), bf16), V((D, F), bf16), V((D, F), bf16), V((F, D), bf16),
        V((16, D), bf16), V((16, D), f32), V((4, NT, 320, 128), u32), V((3, NT, D // 2, 128), u32), V((NT, D // 2, 128), u32),
    ]
    scratch += [V((BM, D), bf16)] * NB + [V((BM, D), bf16)] * NB + [V((NT, BM // 2, 128), u32)] * NB
    scratch += [V((NT, BM, 128), f32)] * NB + [V((NT, HALO + BM, 128), f32)] * (2 * NB)
    scratch += [V((NT, BM, 128), f32) if RC == 8 else V((NT, BM // 2, 128), u32)] * NB + [V((BM, D), f32)] * NB
    scratch += [pltpu.SemaphoreType.DMA((NB,)), pltpu.SemaphoreType.DMA((7,)), pltpu.SemaphoreType.DMA((NB,)),
                pltpu.SemaphoreType.DMA(())]
    any_spec = pl.BlockSpec(memory_space=pl.ANY)

    def fn(A_x, A_wqkv, A_wo, B_x, B_w_r, B_w_gate, B_w_up, B_w_down):
        out = pl.pallas_call(
            kernel,
            out_shape=jax.ShapeDtypeStruct((S, D), bf16),
            in_specs=[any_spec, any_spec, any_spec, pl.BlockSpec(memory_space=pltpu.VMEM), any_spec, any_spec, any_spec],
            out_specs=any_spec,
            scratch_shapes=scratch,
            compiler_params=pltpu.CompilerParams(vmem_limit_bytes=100 * 2 ** 20),
        )(A_x.reshape(S, D), A_wqkv, A_wo, B_w_r, B_w_gate, B_w_up, B_w_down)
        return out.reshape(1, S, D)
    return fn


_fn = make(RC=8, order='mm_first')


@jax.jit
def pallas_sequential_preLN__sliding_local_dilated__moe_arch_mod__prompt_kernel(
    A_x, A_wqkv, A_wo, B_x, B_w_r, B_w_gate, B_w_up, B_w_down,
):
    return _fn(A_x, A_wqkv, A_wo, B_x, B_w_r, B_w_gate, B_w_up, B_w_down)
```

```python
import functools, contextlib
import jax
import jax.numpy as jnp
import numpy as np
from jax.experimental import pallas as pl
from jax.experimental.pallas import tpu as pltpu

S, D, H, DH, F = 2048, 640, 32, 20, 1536
WIN, DIL = 8, 2
NT = D // 128
HALO = 16
EPS = 1e-5
LOG2E = 1.4426950408889634
QSCALE = float(DH ** -0.5) * LOG2E
NEG = -1e9 * LOG2E
bf16 = jnp.bfloat16
f32 = jnp.float32
u32 = jnp.uint32


def _ln(x):
    m = jnp.sum(x, axis=1, keepdims=True) * (1.0 / D)
    c = x - m
    v = jnp.sum(c * c, axis=1, keepdims=True) * (1.0 / D)
    return c * jax.lax.rsqrt(v + EPS)


def _permute_rows(tmp, store):
    for kt in range(NT):
        for dd in range(DH // 2):
            for g in range(2):
                a = tmp[kt, pl.ds(g * 160 + dd, 8, stride=20), :]
                b = tmp[kt, pl.ds(g * 160 + dd + 10, 8, stride=20), :]
                lo = (a & jnp.uint32(0xFFFF)) | (b << 16)
                hi = (a >> 16) | (b & jnp.uint32(0xFFFF0000))
                store(kt, (2 * dd) * 16 + g * 8, lo)
                store(kt, (2 * dd + 1) * 16 + g * 8, hi)


def make(sizes=(256,) * 8, RC=8, RCL=16, RCD=16, L1=1, L2=1, lagB=2, spec=True, xwait=None, pro=None, flags=None, order='mm_first', scopes=False, prog=None):
    NB = len(sizes)
    offs = [sum(sizes[:i]) for i in range(NB)]
    assert sum(sizes) == S

    def kernel(x_hbm, wqkv_hbm, wo_hbm, wr_ref, wg_hbm, wu_hbm, wd_hbm, out_hbm, *scr):
        scr = list(scr)
        def take(n):
            r = scr[:n]; del scr[:n]; return r
        wqkv_v, wo_v, wg_v, wu_v, wd_v, patch_v, y_v, tmp, wp, wop, h_s = take(11)
        x_v = take(NB); out_v = take(NB); xn_s = take(NB); q_s = take(NB); k_s = take(NB); v_s = take(NB); o_s = take(NB)
        sem_x, sem_w, sem_o, sem_p = take(4)

        def cp_x(i):
            return pltpu.make_async_copy(x_hbm.at[pl.ds(offs[i], sizes[i])], x_v[i], sem_x.at[i])

        def cp_w(t):
            return pltpu.make_async_copy(wqkv_hbm.at[:, pl.ds(t * D, D)], wqkv_v.at[:, pl.ds(t * D, D)], sem_w.at[t])

        def cp(name):
            if name.isdigit( ):
                return cp_x(int(name))
            if name in "qkv":
                return cp_w("qkv".index(name))
            src, dst, s = {'o': (wo_hbm, wo_v, 3), 'g': (wg_hbm, wg_v, 4), 'u': (wu_hbm, wu_v, 5), 'd': (wd_hbm, wd_v, 6)}[name]
            return pltpu.make_async_copy(src, dst, sem_w.at[s])

        def start(names):
            for n in names: cp(n).start()

        def wait(names):
            for n in names: cp(n).wait()

        def cp_o(i):
            return pltpu.make_async_copy(out_v[i], out_hbm.at[pl.ds(offs[i], sizes[i])], sem_o.at[i])

        for t in range(NT):
            k_s[0][t, pl.ds(0, HALO), :] = jnp.zeros((HALO, 128), f32)
            v_s[0][t, pl.ds(0, HALO), :] = jnp.zeros((HALO, 128), f32)

        wr = wr_ref[...].astype(f32).reshape(1, D)

        def prep(name):
            if name == 'o':
                t = 3
                for kt in range(NT):
                    tmp[3, kt] = pltpu.bitcast(wo_v[:, pl.ds(kt * 128, 128)], u32)
                def store(kt, r, val):
                    wop[kt, pl.ds(r, 8), :] = val
            else:
                t = "qkv".index(name)
                for kt in range(NT):
                    blk = wqkv_v[pl.ds(kt * 128, 128), pl.ds(t * D, D)]
                    tmp[t, kt] = pltpu.bitcast(blk.T, u32)
                def store(kt, r, val):
                    wp[t, kt, pl.ds(r, 8), :] = val
            _permute_rows(tmp.at[t], store)

        def ln(i, cs=None):
            for c in (range(sizes[i] // RCL) if cs is None else cs):
                r0 = c * RCL
                xx = x_v[i][pl.ds(r0, RCL), :].astype(f32)
                xn = _ln(xx)
                for t in range(NT):
                    xn_s[i][t, pl.ds(r0, RCL), :] = xn[:, t * 128:(t + 1) * 128]

        def cat(ref, *idx):
            ps = [ref[(*idx, t)] for t in range(NT)]
            if ps[0].dtype == u32:
                return jnp.concatenate([pltpu.bitcast(p, bf16) for p in ps], axis=1)
            return jnp.concatenate(ps, axis=1).astype(bf16)

        def A(i, t3):
            res = jax.lax.dot_general(cat(xn_s[i]), cat(wp, t3), (((1,), (1,)), ((), ())), preferred_element_type=f32)
            dst = (q_s, k_s, v_s)[t3]
            for t in range(NT):
                if t3 == 0:
                    dst[i][t] = res[:, t * 128:(t + 1) * 128]
                else:
                    dst[i][t, pl.ds(HALO, sizes[i]), :] = res[:, t * 128:(t + 1) * 128]
                    if i + 1 < NB:
                        dst[i + 1][t, pl.ds(0, HALO), :] = res[sizes[i] - HALO:, t * 128:(t + 1) * 128]

        def C(i):
            res = jnp.dot(cat(o_s[i]), cat(wop), preferred_element_type=f32)
            h_s[pl.ds(offs[i], sizes[i]), :] = res + x_v[i][...].astype(f32)

        def b1(i, r0):
            q = [q_s[i][t, pl.ds(r0, RC), :] for t in range(NT)]
            accs = []
            for j in range(WIN):
                acc = None
                for t in range(NT):
                    p = q[t] * k_s[i][t, pl.ds(HALO + r0 - DIL * j, RC), :]
                    acc = p if acc is None else acc + p
                accs.append(acc)
            return [(a, pltpu.roll(a, 64, 1)) for a in accs]

        def b2(st):
            out = []
            for (a, r) in st:
                s = a + r
                out.append((s, pltpu.roll(s, 32, 1)))
            return out

        def b3(i, r0, st):
            L = []
            for j in range(WIN):
                acc = (st[j][0] + st[j][1]) * QSCALE
                if offs[i] + r0 < DIL * j:
                    row = jax.lax.broadcasted_iota(jnp.int32, (RC, 128), 0) + (offs[i] + r0)
                    acc = jnp.where(row >= DIL * j, acc, NEG)
                L.append(acc)
            m = L[0]
            for j in range(1, WIN):
                m = jnp.maximum(m, L[j])
            e = [jnp.exp2(l - m) for l in L]
            ssum = e[0]
            for j in range(1, WIN):
                ssum = ssum + e[j]
            inv = pl.reciprocal(ssum, approx=True)
            inv = inv * (2.0 - ssum * inv)
            for t in range(NT):
                acc = None
                for j in range(WIN):
                    p = e[j] * v_s[i][t, pl.ds(HALO + r0 - DIL * j, RC), :]
                    acc = p if acc is None else acc + p
                if RC == 8:
                    o_s[i][t, pl.ds(r0, RC), :] = acc * inv
                else:
                    o_s[i][t, pl.ds(r0 // 2, RC // 2), :] = pltpu.bitcast((acc * inv).astype(bf16), u32)

        s1 = {}; s2 = {}
        chunks = [(i, r0) for i in range(NB) for r0 in range(0, sizes[i], RC)]
        cstart = [sum(sizes[:i]) // RC for i in range(NB + 1)]
        nbs = len(chunks) + L1 + L2
        def b_step(g):
            n = len(chunks)
            if 0 <= g < n:
                s1[g] = b1(*chunks[g])
            if 0 <= g - L1 < n:
                s2[g - L1] = b2(s1.pop(g - L1))
            if 0 <= g - L1 - L2 < n:
                gg = g - L1 - L2
                b3(*chunks[gg], s2.pop(gg))

        best = [None, None]

        def Dst(i, cs):
            for c in cs:
                r0 = c * RCD
                hh = h_s[pl.ds(offs[i] + r0, RCD), :]
                xn2 = _ln(hh)
                out_v[i][pl.ds(r0, RCD), :] = (hh + xn2).astype(bf16)
                r = jnp.sum(xn2 * wr, axis=1, keepdims=True)
                g0 = float(offs[i] + r0)
                if best[0] is None:
                    best[0] = r
                    best[1] = jnp.full((RCD, 1), g0, f32)
                else:
                    upd = r > best[0]
                    best[0] = jnp.where(upd, r, best[0])
                    best[1] = jnp.where(upd, g0, best[1])

        def argmax():
            m = jnp.max(best[0], axis=0, keepdims=True)
            rowi = jax.lax.broadcasted_iota(jnp.int32, (RCD, 1), 0).astype(f32)
            cand = jnp.where(best[0] == m, best[1] + rowi, float(S))
            idx = jnp.min(cand).astype(jnp.int32)
            return jnp.clip(idx, 0, S - 1)

        def ffn(idx):
            base = pl.multiple_of((idx // 16) * 16, 16)
            hh = h_s[pl.ds(base, 16), :]
            xn2 = _ln(hh)
            r = jnp.sum(xn2 * wr, axis=1, keepdims=True)
            xb = xn2.astype(bf16)
            g = jnp.dot(xb, wg_v[...], preferred_element_type=f32)
            u = jnp.dot(xb, wu_v[...], preferred_element_type=f32)
            a = (g * jax.nn.sigmoid(g) * u).astype(bf16)
            y = jnp.dot(a, wd_v[...], preferred_element_type=f32) * jax.nn.sigmoid(r)
            rowsel = jax.lax.broadcasted_iota(jnp.int32, (16, D), 0) == (idx - base)
            patch_v[...] = (hh + xn2 + jnp.where(rowsel, y, 0.0)).astype(bf16)

        sc = (lambda n: jax.named_scope(n)) if scopes else (lambda n: contextlib.nullcontext())
        st = {'spec': None}

        def Bblk(i):
            n_ = sizes[i] // RC
            t1 = {}; t2 = {}
            for c in range(n_ + 2):
                if c < n_: t1[c] = b1(i, c * RC)
                if 0 <= c - 1 < n_: t2[c - 1] = b2(t1.pop(c - 1))
                if 0 <= c - 2 < n_: b3(i, (c - 2) * RC, t2.pop(c - 2))

        def emit(tk):
            op, arg = tk[0], tk[1:]
            if op == '+': start(arg)
            elif op == '-': wait(arg)
            elif op == 'p': prep(arg)
            elif op == 'l': ln(int(arg))
            elif op == 'A': A(int(arg[1:]), "qkv".index(arg[0]))
            elif op == 'B': Bblk(int(arg))
            elif op == 'C': C(int(arg))
            elif op == 'D': Dst(int(arg), range(sizes[int(arg)] // RCD))
            elif op == 'o': cp_o(int(arg)).start()
            elif op == 'S':
                st['spec'] = argmax()
                ffn(st['spec'])
            else: raise ValueError(tk)

        for n_, region in enumerate(prog.split('|')):
            with sc("r%02d_%s" % (n_, region.strip().replace(' ', '_')[:30])):
                for tk in region.split():
                    emit(tk)

        with sc("tail"):
            idx = argmax()
            if st['spec'] is not None:
                @pl.when(idx != st['spec'])
                def _():
                    ffn(idx)
            else:
                ffn(idx)
            base = pl.multiple_of((idx // 16) * 16, 16)
            for i in range(NB):
                cp_o(i).wait()
            cpp = pltpu.make_async_copy(patch_v, out_hbm.at[pl.ds(base, 16)], sem_p)
            cpp.start()
            cpp.wait()

    V = pltpu.VMEM
    scratch = [
        V((D, 3 * D), bf16), V((D, D), bf16), V((D, F), bf16), V((D, F), bf16), V((F, D), bf16),
        V((16, D), bf16), V((16, D), f32), V((4, NT, 320, 128), u32), V((3, NT, D // 2, 128), u32),
        V((NT, D // 2, 128), u32), V((S, D), f32),
    ]
    scratch += [V((b, D), bf16) for b in sizes] * 2 + [V((NT, b, 128), f32) for b in sizes] * 2
    scratch += [V((NT, HALO + b, 128), f32) for b in sizes] * 2
    scratch += [(V((NT, b, 128), f32) if RC == 8 else V((NT, b // 2, 128), u32)) for b in sizes]
    scratch += [pltpu.SemaphoreType.DMA((NB,)), pltpu.SemaphoreType.DMA((7,)), pltpu.SemaphoreType.DMA((NB,)),
                pltpu.SemaphoreType.DMA(())]
    any_spec = pl.BlockSpec(memory_space=pl.ANY)

    def fn(A_x, A_wqkv, A_wo, B_x, B_w_r, B_w_gate, B_w_up, B_w_down):
        out = pl.pallas_call(
            kernel,
            out_shape=jax.ShapeDtypeStruct((S, D), bf16),
            in_specs=[any_spec, any_spec, any_spec, pl.BlockSpec(memory_space=pltpu.VMEM), any_spec, any_spec, any_spec],
            out_specs=any_spec,
            scratch_shapes=scratch,
            compiler_params=pltpu.CompilerParams(vmem_limit_bytes=100 * 2 ** 20, **({'flags': flags} if flags else {})),
        )(A_x.reshape(S, D), A_wqkv, A_wo, B_w_r, B_w_gate, B_w_up, B_w_down)
        return out.reshape(1, S, D)
    return fn


_PROG = '+q01 -q0 +kv2o l0 pq -1 l1 Aq0 -k Aq1 pk -v +345678gud Ak0 pv -2o Av0 po l2 Ak1 Av1 B0 -3 Aq2 Ak2 Av2 C0 B1 l3 -4 Aq3 Ak3 Av3 C1 B2 l4 D0 o0 -5 Aq4 Ak4 Av4 C2 B3 l5 D1 o1 -6 Aq5 Ak5 Av5 C3 B4 l6 D2 o2 -7 Aq6 Ak6 Av6 C4 B5 l7 D3 o3 -8 Aq7 Ak7 Av7 C5 B6 l8 D4 o4 Aq8 Ak8 Av8 C6 B7 D5 o5 C7 B8 D6 o6 C8 D7 o7 -gud S D8 o8'
_fn = make(sizes=(256,) * 7 + (128,) * 2, prog=_PROG, RCL=64, RCD=64,
           flags={"XLA_TPU_EVENLY_DISTRIBUTE_CRITICAL_NODES": True})


@jax.jit
def pallas_sequential_preLN__sliding_local_dilated__moe_arch_mod__prompt_kernel(
    A_x, A_wqkv, A_wo, B_x, B_w_r, B_w_gate, B_w_up, B_w_down,
):
    return _fn(A_x, A_wqkv, A_wo, B_x, B_w_r, B_w_gate, B_w_up, B_w_down)
```
